```python
import os as _os
_os.environ.setdefault("JAX_PLATFORMS", "cpu")
import jax
import jax.numpy as jnp

def _softmax(x, axis=-1):
    return jax.nn.softmax(x, axis=axis)
def _gelu(x):
    return jax.nn.gelu(x, approximate=True)
def _silu(x):
    return jax.nn.silu(x)
def _sigmoid(x):
    return jax.nn.sigmoid(x)
def _layernorm(x, axis=-1, eps=1e-5):
    m = jnp.mean(x, axis=axis, keepdims=True)
    v = jnp.var(x, axis=axis, keepdims=True)
    return (x - m) / jnp.sqrt(v + eps)
def _scatter_add(tgt, idx, src, axis=0):
    return tgt.at[idx].add(src)
def _segment_sum(src, seg, n):
    return jax.ops.segment_sum(src, seg, n)
class _Rng:
    def __init__(self, key):
        self._k = key
    def _next(self):
        self._k, sub = jax.random.split(self._k)
        return sub
    def normal(self, shape):
        return jax.random.normal(self._next(), shape, dtype=jnp.bfloat16)
    def randint(self, lo, hi, shape):
        return jax.random.randint(self._next(), shape, lo, hi, dtype=jnp.int32)
    def uniform(self, shape, lo=0.0, hi=1.0):
        return jax.random.uniform(self._next(), shape, jnp.bfloat16, lo, hi)
    def permutation(self, n):
        return jax.random.permutation(self._next(), n)


kernel_name = 'concat_heads__sliding_block__grouped_kv_mqa__prompt'

def setup_inputs():
    _rng = _Rng(jax.random.key(int.from_bytes(__import__("os").urandom(4), "little")))
    _w = (lambda a: (lambda t: t.astype(jnp.bfloat16) if jnp.issubdtype(t.dtype, jnp.floating) else t)(jnp.asarray(a)))
    def _A_setup():
        B, S, D = 1, 2048, 576
        return {
            "x": _w((lambda *s: _rng.normal(s) * 0.2)(B, S, D)),
            "wqkv": _w((lambda *s: _rng.normal(s) * 0.2)(D, 3 * D)),
            "wo": _w((lambda *s: _rng.normal(s) * 0.05)(D, D)),
        }
    _A_in = _A_setup()

    def _B_setup():
        B, S, D, H = 1, 2048, 576, 32
        Dh = D // H
        return {
            "x": _w((lambda *s: _rng.normal(s) * 0.05)(B, S, D)),
            "wq": _w((lambda *s: _rng.normal(s) * 1.6)(D, H * Dh)),
            "wk": _w((lambda *s: _rng.normal(s) * 1.6)(D, Dh)),
            "wv": _w((lambda *s: _rng.normal(s) * 0.1)(D, Dh)),
            "wo": _w((lambda *s: _rng.normal(s) * 0.1)(H * Dh, D)),
        }
    _B_in = _B_setup()

    return {
        "A_x": _A_in["x"],
        "A_wqkv": _A_in["wqkv"],
        "A_wo": _A_in["wo"],
        "B_x": _B_in["x"],
        "B_wq": _B_in["wq"],
        "B_wk": _B_in["wk"],
        "B_wv": _B_in["wv"],
        "B_wo": _B_in["wo"],
    }

def reference(A_x, A_wqkv, A_wo, B_x, B_wq, B_wk, B_wv, B_wo):
    def _A_ref(x, wqkv, wo):
        B, S, D = x.shape
        H = 32; Dh = D // H; W = 256
        qkv = (lambda x, *d: x.transpose(*d))((x @ wqkv).reshape(B, S, 3, H, Dh), 2, 0, 3, 1, 4)
        q, k, v = qkv[0], qkv[1], qkv[2]
        scores = jnp.einsum("bhqd,bhkd->bhqk", q, k) * (Dh ** -0.5)
        idx = jnp.arange(S)
        mask = (idx[:, None] - idx[None, :] >= 0) & (idx[:, None] - idx[None, :] < W)
        scores = jnp.where(mask[None, None], scores, -1e9)
        p = _softmax(scores, axis=-1)
        o = jnp.einsum("bhqk,bhkd->bhqd", p, v)
        return (lambda x, *d: x.transpose(*d))(o, 0, 2, 1, 3).reshape(B, S, D) @ wo

    def _B_ref(x, wq, wk, wv, wo):
        B, S, D = x.shape
        H = 32
        Dh = D // H
        q = (lambda x, *d: x.transpose(*d))((x @ wq).reshape(B, S, H, Dh), 0, 2, 1, 3)
        k = x @ wk
        v = x @ wv
        scores = jnp.einsum("bhqd,bkd->bhqk", q, k) * (Dh ** -0.5)
        p = _softmax(scores, axis=-1)
        o = jnp.einsum("bhqk,bkd->bhqd", p, v)
        return (lambda x, *d: x.transpose(*d))(o, 0, 2, 1, 3).reshape(B, S, H * Dh) @ wo

    a = _A_ref(A_x, A_wqkv, A_wo)
    b = _B_ref(B_x, B_wq, B_wk, B_wv, B_wo)
    return jnp.concatenate([a, b], axis=-1)
```

```python
import functools
import math

import numpy as np
import jax
import jax.numpy as jnp
from jax import lax
import jax.experimental.pallas as pl
import jax.experimental.pallas.tpu as pltpu

BF = jnp.bfloat16
F32 = jnp.float32

S = 2048
D = 576
H = 32
DH = 18
WIN = 256
NSLAB = 5
DP = NSLAB * 128
QB = 512
NQB = S // QB
TPS = QB // 128
DV = 24
TRIM = 48
BK = 128
NEG = -1e30
QSCALE = (DH ** -0.5) * math.log2(math.e)


def _slab_rows(p, base, j):
    if j < NSLAB - 1:
        return p[base + 126 * j: base + 126 * j + 128, :], 0
    return p[base + 450 + TRIM: base + 450 + 128, :], TRIM


def _nn(a, b):
    return jnp.dot(a, b, preferred_element_type=F32)


def _head_rows(qs, i):
    qi = pltpu.bitcast(qs, jnp.int32)
    r = lax.broadcasted_iota(jnp.int32, qi.shape, 0) - (DH // 2) * i
    keep = (r >= 0) & (r < DH // 2)
    return pltpu.bitcast(jnp.where(keep, qi, 0), BF)


def _head_rows_static(qs, i):
    n = qs.shape[1]
    r0 = 16 * i
    win = pltpu.bitcast(qs[r0:r0 + 32, :], jnp.int32)
    r = lax.broadcasted_iota(jnp.int32, win.shape, 0) - i
    win = pltpu.bitcast(jnp.where((r >= 0) & (r < DH // 2), win, 0), BF)
    parts = []
    if r0:
        parts.append(jnp.zeros((r0, n), BF))
    parts.append(win)
    if r0 + 32 < 128:
        parts.append(jnp.zeros((128 - r0 - 32, n), BF))
    return jnp.concatenate(parts, axis=0) if len(parts) > 1 else win


def _kernel(z_ref, xa_hbm, xb_hbm, wqkv_hbm, woa_hbm, wqb_hbm, wkb_hbm, wvb_hbm, wob_hbm,
            out_hbm,
            xa, xb, wqkv, woa, wqb, wkb, wvb, wob, sems, osems,
            wta, wota, wotb, ka, vta, qta, qtb, kb, vtb, ota, otb,
            bias, sa0, sa1, sb0, sb1, outv):
    z0 = pl.multiple_of(z_ref[0], 128)
    z1 = pl.multiple_of(z_ref[1], 128)
    z2 = pl.multiple_of(z_ref[2], 128)
    z3 = pl.multiple_of(z_ref[3], 128)

    def cols(c):
        return slice(c * QB, (c + 1) * QB)

    def dma(n):
        srcs = (wkb_hbm, wvb_hbm, wqb_hbm) + tuple(
            xb_hbm.at[:, cols(c)] for c in range(NQB)) + (wqkv_hbm,) + tuple(
            xa_hbm.at[:, cols(c)] for c in range(NQB)) + (woa_hbm, wob_hbm)
        dsts = (wkb, wvb, wqb) + tuple(
            xb.at[:, cols(c)] for c in range(NQB)) + (wqkv,) + tuple(
            xa.at[:, cols(c)] for c in range(NQB)) + (woa, wob)
        return pltpu.make_async_copy(srcs[n], dsts[n], sems.at[n])

    D_WK, D_WV, D_WQ, D_XB, D_WQKV, D_XA, D_WOA, D_WOB = 0, 1, 2, 3, 7, 8, 12, 13
    for n in range(14):
        dma(n).start()

    kr = lax.broadcasted_iota(jnp.int32, (3 * 128, 128), 0)
    qi = lax.broadcasted_iota(jnp.int32, (3 * 128, 128), 1)
    for v in range(3):
        ok = (kr > qi) & (kr <= WIN + qi) & (kr >= WIN - 128 * v)
        bias[v] = jnp.where(ok, 0.0, NEG)
    ka[:, 0:WIN, :] = jnp.zeros((NSLAB, WIN, 128), BF)
    vta[:, 0:WIN] = jnp.zeros((D, WIN), F32)
    qtb[NSLAB - 1, 0:TRIM, :] = jnp.zeros((TRIM, S), BF)
    ota[...] = jnp.zeros(ota.shape, F32)
    otb[...] = jnp.zeros(otb.shape, F32)

    r = lax.broadcasted_iota(jnp.int32, (128, DH), 0)
    c = lax.broadcasted_iota(jnp.int32, (128, DH), 1)
    rep = ((r % DH == c) & (r < 126)).astype(BF)
    place = ((r % DV - 2 * (r // DV) == c) & (r < 4 * DV)).astype(BF)
    dma(D_WK).wait()
    wk_rep = _nn(rep, wkb[...]).astype(BF)
    dma(D_WV).wait()
    wv_var = _nn(place, wvb[...]).astype(BF)[0:4 * DV, :]
    dma(D_WQ).wait()
    wtb = jnp.concatenate([wqb[...].T, wk_rep, wv_var], axis=0)
    rr = lax.broadcasted_iota(jnp.int32, (DV, QB), 0)
    for cc in range(NQB):
        dma(D_XB + cc).wait()
        pb = _nn(wtb, xb[:, cols(cc)])
        for j in range(NSLAB):
            q, r0 = _slab_rows(pb, 0, j)
            qtb[j, r0:128, cols(cc)] = (q * QSCALE).astype(BF)
        kb[cols(cc), :] = pb[D:D + 128, :].astype(BF).T
        vt = pb[D + 128:, :].astype(BF).astype(F32)
        for v in range(4):
            vtb[v, :, cols(cc)] = jnp.where(rr == (2 * v + DH) % DV, 1.0, vt[v * DV:(v + 1) * DV, :])
        if cc == 1:
            dma(D_WQKV).wait()
            wta[0:D, :] = wqkv[:, 0:D].T
            wta[D:2 * D, :] = wqkv[:, D:2 * D].T
        if cc == 2:
            wta[2 * D:3 * D, :] = wqkv[:, 2 * D:3 * D].T
        if cc == 3:
            dma(D_WOA).wait()
            wota[...] = woa[...].T
            dma(D_WOB).wait()
            wotb[...] = wob[...].T
    for cc in range(NQB):
        dma(D_XA + cc).wait()

    def a_proj(cc, carry):
        x0 = pl.multiple_of(cc * QB, QB)
        k0 = pl.multiple_of(WIN + cc * QB, 256)
        pa = _nn(wta[...], xa[:, pl.ds(x0, QB)])
        for j in range(NSLAB):
            q, r0 = _slab_rows(pa, 0, j)
            qta[j, r0:128, pl.ds(x0, QB)] = (q * QSCALE).astype(BF)
            k, _ = _slab_rows(pa, D, j)
            k = k.astype(BF)
            if r0:
                k = jnp.concatenate([jnp.zeros((r0, QB), BF), k], axis=0)
            ka[j, pl.ds(k0, QB), :] = k.T
        vta[:, pl.ds(k0, QB)] = pa[2 * D:3 * D, :].astype(BF).astype(F32)
        return carry

    lax.fori_loop(0, NQB, a_proj, 0)

    rowv = lax.broadcasted_iota(jnp.int32, (DV, 3 * 128), 0)
    rows = lax.broadcasted_iota(jnp.int32, (DV, 128), 0)

    def a_qk(j, t, heads, s_ref, zn):
        t0 = pl.multiple_of(t * 128, 128)
        lo, hi = heads[0] * 128, (heads[-1] + 1) * 128
        qs = qta[j, :, pl.ds(t0, 128)]
        w = jnp.concatenate([_head_rows_static(qs, i) for i in heads], axis=1)
        bt = bias[jnp.minimum(t, 2)]
        st = _nn(ka[j, pl.ds(t0, 3 * 128), :], w) + jnp.concatenate([bt] * len(heads), axis=1)
        s_ref[pl.ds(zn, 3 * 128), lo:hi] = st
        m = jnp.max(st.reshape(3 * 16, 8, hi - lo), axis=0)
        m = jnp.max(m, axis=0, keepdims=True)
        if lo:
            m = jnp.concatenate([jnp.zeros((1, lo), F32), m], axis=1)
        return m

    def a_pv(j, t, heads, s_ref, zc, m):
        t0 = pl.multiple_of(t * 128, 128)
        h0 = jnp.where(j == NSLAB - 1, 25, 7 * j)
        for i in heads:
            hc = slice(i * 128, (i + 1) * 128)
            p = jnp.exp2(s_ref[pl.ds(zc, 3 * 128), hc] - m[:, hc]).astype(BF)
            h = h0 + i
            off = (2 * h) % 8
            r0 = pl.multiple_of(((DH * h) // 8) * 8, 8)
            lpos = (off + DH) % DV
            vw = vta[pl.ds(r0, DV), pl.ds(t0, 3 * 128)]
            vw = jnp.where(rowv == lpos, 1.0, vw)
            acc = _nn(vw, p)
            l = jnp.sum(jnp.where(rows == lpos, acc, 0.0), axis=0, keepdims=True)
            val = acc * (1.0 / l)
            d = rows - off
            keep = (d >= 0) & (d < DH)
            old = ota[pl.ds(r0, DV), pl.ds(t0, 128)]
            ota[pl.ds(r0, DV), pl.ds(t0, 128)] = jnp.where(keep, val, old)

    def a_unit(j, tg, m, jn, tgn, heads):
        t = tg * TPS
        m1 = a_qk(j, t + 1, heads, sa1, z1)
        a_pv(j, t, heads, sa0, z0, m)
        m2 = a_qk(j, t + 2, heads, sa0, z3)
        a_pv(j, t + 1, heads, sa1, z2, m1)
        m3 = a_qk(j, t + 3, heads, sa1, z1)
        a_pv(j, t + 2, heads, sa0, z0, m2)
        m0 = a_qk(jn, tgn * TPS, heads, sa0, z3)
        a_pv(j, t + 3, heads, sa1, z2, m3)
        return m0

    all7 = tuple(range(7))
    last4 = (3, 4, 5, 6)
    m_a = a_qk(0, 0, all7, sa0, 0)

    def a_body7(u, m):
        un = u + 1
        return a_unit(u // NQB, u % NQB, m, un // NQB, un % NQB, all7)

    m_a = lax.fori_loop(0, (NSLAB - 1) * NQB, a_body7, m_a)

    def a_body4(tg, m):
        return a_unit(NSLAB - 1, tg, m, NSLAB - 1, jnp.minimum(tg + 1, NQB - 1), last4)

    lax.fori_loop(0, NQB, a_body4, m_a)

    row24 = lax.broadcasted_iota(jnp.int32, (DV, QB), 0)

    def b_item(item):
        item = jnp.minimum(item, NQB * H - 1)
        h = item % H
        q0 = pl.multiple_of((item // H) * QB, QB)
        j = jnp.minimum(h // 7, 4)
        i = h - jnp.where(j == 4, 25, 7 * j)
        return j, i, q0

    def b_weights(item):
        j, i, q0 = b_item(item)
        return _head_rows(qtb[j, :, pl.ds(q0, QB)], i)

    def b_qk_chunk(c, wq, s_ref, zn, m):
        st = _nn(kb[c * BK:(c + 1) * BK, :], wq)
        s_ref[pl.ds(zn + c * BK, BK), :] = st
        return jnp.maximum(m, jnp.max(st.reshape(BK // 8, 8, QB), axis=0))

    def b_finalize(item, acc):
        _, _, q0 = b_item(item)
        h = item % H
        off = (2 * h) % 8
        r0 = pl.multiple_of(((DH * h) // 8) * 8, 8)
        lpos = (off + DH) % DV
        l = jnp.sum(jnp.where(row24 == lpos, acc, 0.0), axis=0, keepdims=True)
        val = acc * (1.0 / l)
        d = row24 - off
        keep = (d >= 0) & (d < DH)
        old = otb[pl.ds(r0, DV), pl.ds(q0, QB)]
        otb[pl.ds(r0, DV), pl.ds(q0, QB)] = jnp.where(keep, val, old)

    def b_step(item, m_cur, s_cur, s_nxt, zc, zn):
        var = item % 4
        wq = b_weights(item + 1)
        m_next = jnp.full((8, QB), NEG, F32)
        acc = jnp.zeros((DV, QB), F32)
        for c in range(S // BK):
            m_next = b_qk_chunk(c, wq, s_nxt, zn, m_next)
            p = jnp.exp2(s_cur[pl.ds(zc + c * BK, BK), :] - m_cur)
            acc = acc + _nn(vtb[var, :, c * BK:(c + 1) * BK], p.astype(BF))
        b_finalize(item, acc)
        return jnp.max(m_next, axis=0, keepdims=True)

    wq0 = b_weights(0)
    m_b = jnp.full((8, QB), NEG, F32)
    for cc in range(S // BK):
        m_b = b_qk_chunk(cc, wq0, sb0, 0, m_b)
    m_b = jnp.max(m_b, axis=0, keepdims=True)

    def b_body(u, m):
        m = b_step(2 * u, m, sb0, sb1, z0, z1)
        m = b_step(2 * u + 1, m, sb1, sb0, z2, z3)
        return m

    lax.fori_loop(0, NQB * H // 2, b_body, m_b)

    def out_dma(cc):
        return pltpu.make_async_copy(outv.at[cc], out_hbm.at[cols(cc), :], osems.at[cc])

    for cc in range(NQB):
        res = []
        for wo, ot in ((wota, ota), (wotb, otb)):
            o = ot[:, cols(cc)].astype(BF)
            res.append(_nn(wo[...], o).astype(BF))
        outv[cc] = jnp.concatenate(res, axis=0).T
        out_dma(cc).start()
    for cc in range(NQB):
        out_dma(cc).wait()


@jax.jit
def pallas_concat_heads__sliding_block__grouped_kv_mqa__prompt_kernel(
    A_x: jax.Array,
    A_wqkv: jax.Array,
    A_wo: jax.Array,
    B_x: jax.Array,
    B_wq: jax.Array,
    B_wk: jax.Array,
    B_wv: jax.Array,
    B_wo: jax.Array,
):
    xa = A_x.reshape(S, D).T
    xb = B_x.reshape(S, D).T
    zeros = np.zeros((4,), np.int32)
    hbm = pl.BlockSpec(memory_space=pltpu.HBM)
    scratch = [
        pltpu.VMEM((D, S), BF),
        pltpu.VMEM((D, S), BF),
        pltpu.VMEM((D, 3 * D), BF),
        pltpu.VMEM((D, D), BF),
        pltpu.VMEM((D, D), BF),
        pltpu.VMEM((DH, D), BF),
        pltpu.VMEM((DH, D), BF),
        pltpu.VMEM((D, D), BF),
        pltpu.SemaphoreType.DMA((14,)),
        pltpu.SemaphoreType.DMA((NQB,)),
        pltpu.VMEM((3 * D, D), BF),
        pltpu.VMEM((D, D), BF),
        pltpu.VMEM((D, D), BF),
        pltpu.VMEM((NSLAB, WIN + S, 128), BF),
        pltpu.VMEM((D, WIN + S), F32),
        pltpu.VMEM((NSLAB, 128, S), BF),
        pltpu.VMEM((NSLAB, 128, S), BF),
        pltpu.VMEM((S, 128), BF),
        pltpu.VMEM((4, DV, S), F32),
        pltpu.VMEM((D, S), F32),
        pltpu.VMEM((D, S), F32),
        pltpu.VMEM((3, 3 * 128, 128), F32),
        pltpu.VMEM((3 * 128, 7 * 128), F32),
        pltpu.VMEM((3 * 128, 7 * 128), F32),
        pltpu.VMEM((S, QB), F32),
        pltpu.VMEM((S, QB), F32),
        pltpu.VMEM((NQB, QB, 2 * D), BF),
    ]
    out = pl.pallas_call(
        _kernel,
        in_specs=[pl.BlockSpec(memory_space=pltpu.SMEM)] + [hbm] * 8,
        out_specs=hbm,
        out_shape=jax.ShapeDtypeStruct((S, 2 * D), BF),
        scratch_shapes=scratch,
        compiler_params=pltpu.CompilerParams(vmem_limit_bytes=100 * 1024 * 1024),
    )(zeros, xa, xb, A_wqkv, A_wo, B_wq, B_wk.T, B_wv.T, B_wo)
    return out.reshape(1, S, 2 * D)
```

```python
import functools
import math

import numpy as np
import jax
import jax.numpy as jnp
from jax import lax
import jax.experimental.pallas as pl
import jax.experimental.pallas.tpu as pltpu

BF = jnp.bfloat16
F32 = jnp.float32

S = 2048
D = 576
H = 32
DH = 18
WIN = 256
HG = 4
NG = H // HG
GR = 80
QB = 512
NQB = S // QB
DV = 24
BK = 128
NEG = -1e30
B_UNROLL = 4
NT = S // 128
OUT_TAIL = ((1536, 384), (1920, 128))
QSCALE = (DH ** -0.5) * math.log2(math.e)


def _nn(a, b):
    return jnp.dot(a, b, preferred_element_type=F32)


def _head_rows(qs, k):
    n = qs.shape[1]
    r0 = 16 * k
    win = pltpu.bitcast(qs[r0:r0 + 32, :], jnp.int32)
    r = lax.broadcasted_iota(jnp.int32, win.shape, 0) - k
    win = pltpu.bitcast(jnp.where((r >= 0) & (r < DH // 2), win, 0), BF)
    parts = [jnp.zeros((r0, n), BF)] if r0 else []
    parts.append(win)
    if r0 + 32 < GR:
        parts.append(jnp.zeros((GR - r0 - 32, n), BF))
    return jnp.concatenate(parts, axis=0)


def _kernel(z_ref, xa_hbm, xb_hbm, wqkv_hbm, woa_hbm, wqb_hbm, wkb_hbm, wvb_hbm, wob_hbm,
            out_hbm,
            xa, xb, wqkv, woa, wqb, wkb, wvb, wob, sems, osems,
            wta, wota, wotb, ka, vta, qta, qtb, kb, vtb, ota, otb,
            bias, sa0, sa1, sa2, sa3, sb0, sb1, outv):
    def cols(c):
        return slice(c * QB, (c + 1) * QB)

    def dma(n):
        srcs = (wkb_hbm, wvb_hbm, wqb_hbm) + tuple(
            xb_hbm.at[:, cols(c)] for c in range(NQB)) + (wqkv_hbm, woa_hbm, wob_hbm) + tuple(
            xa_hbm.at[:, cols(c)] for c in range(NQB))
        dsts = (wkb, wvb, wqb) + tuple(
            xb.at[:, cols(c)] for c in range(NQB)) + (wqkv, woa, wob) + tuple(
            xa.at[:, cols(c)] for c in range(NQB))
        return pltpu.make_async_copy(srcs[n], dsts[n], sems.at[n])

    D_WK, D_WV, D_WQ, D_XB, D_WQKV, D_WOA, D_WOB, D_XA = 0, 1, 2, 3, 7, 8, 9, 10
    for n in range(14):
        dma(n).start()

    kr = lax.broadcasted_iota(jnp.int32, (3 * 128, 128), 0)
    qi = lax.broadcasted_iota(jnp.int32, (3 * 128, 128), 1)
    bias[...] = jnp.where((kr > qi) & (kr <= WIN + qi), 0.0, NEG)

    r = lax.broadcasted_iota(jnp.int32, (2 * DV, DH), 0)
    c = lax.broadcasted_iota(jnp.int32, (2 * DV, DH), 1)
    dma(D_WK).wait()
    dma(D_WV).wait()
    wkv = (_nn((r == c).astype(BF), wkb[...]) + _nn((r == c + DV).astype(BF), wvb[...])).astype(BF)
    dma(D_WQ).wait()
    wtb = jnp.concatenate([wqb[...].T, wkv], axis=0)
    rr = lax.broadcasted_iota(jnp.int32, (DV, QB), 0)
    for cc in range(NQB):
        dma(D_XB + cc).wait()
        if cc == 2:
            dma(D_WQKV).wait()
        if cc == 3:
            dma(D_WOA).wait()
            dma(D_WOB).wait()
        pb = _nn(wtb, xb[:, cols(cc)])
        if cc == 2:
            wta[0:D, :] = wqkv[:, 0:D].T
            wta[D:2 * D, :] = wqkv[:, D:2 * D].T
        if cc == 3:
            wta[2 * D:3 * D, :] = wqkv[:, 2 * D:3 * D].T
            wota[...] = woa[...].T
            wotb[...] = wob[...].T
        ota[:, cols(cc)] = jnp.zeros((D, QB), F32)
        otb[:, cols(cc)] = jnp.zeros((D, QB), F32)
        for g in range(NG):
            qtb[g, :, cols(cc)] = (pb[72 * g:72 * g + GR, :] * QSCALE).astype(BF)
        kt = pb[D:D + DH, :]
        kt = jnp.concatenate([kt] * HG + [jnp.zeros((GR - HG * DH, QB), F32)], axis=0)
        kb[cols(cc), :] = kt.astype(BF).T
        vt = jnp.where(rr == DH, 1.0, pb[D + DV:D + 2 * DV, :].astype(BF).astype(F32))
        for v in range(HG):
            vtb[v, :, cols(cc)] = jnp.concatenate([vt[DV - 2 * v:, :], vt[:DV - 2 * v, :]], axis=0) if v else vt
    for cc in range(NQB):
        dma(D_XA + cc).wait()

    def a_proj(cc, carry):
        x0 = pl.multiple_of(cc * QB, QB)
        pa = _nn(wta[...], xa[:, pl.ds(x0, QB)])
        for g in range(NG):
            qta[g, :, pl.ds(x0, QB)] = (pa[72 * g:72 * g + GR, :] * QSCALE).astype(BF)
            ka[g, pl.ds(x0, QB), :] = pa[D + 72 * g:D + 72 * g + GR, :].astype(BF).T
        vta[:, pl.ds(x0, QB)] = pa[2 * D:3 * D, :].astype(BF).astype(F32)
        return carry

    lax.fori_loop(0, NQB, a_proj, 0)

    rows = lax.broadcasted_iota(jnp.int32, (DV, 128), 0)

    def a_qk(g, t, s_ref):
        t0 = t * 128
        nt = min(t + 1, 3)
        skip = 3 - nt
        qs = qta[g, :, t0:t0 + 128]
        w = jnp.concatenate([_head_rows(qs, k) for k in range(HG)], axis=1)
        st = _nn(ka[g, t0 + 128 - nt * 128:t0 + 128, :], w)
        tiles = []
        for n in range(nt):
            tile = st[n * 128:(n + 1) * 128, :]
            if n + skip != 1:
                bt = bias[(n + skip) * 128:(n + skip + 1) * 128, :]
                tile = tile + jnp.concatenate([bt] * HG, axis=1)
            tiles.append(tile)
        st = jnp.concatenate(tiles, axis=0) if nt > 1 else tile
        s_ref[skip * 128:, :] = st
        m = jnp.max(st.reshape(nt * 16, 8, HG * 128), axis=0)
        return jnp.max(m, axis=0, keepdims=True)

    def a_pv(g, t, s_ref, m):
        t0 = t * 128
        nk = min(t + 1, 3) * 128
        skip = 3 - nk // 128
        rowv = lax.broadcasted_iota(jnp.int32, (DV, nk), 0)
        for k in range(HG):
            hc = slice(k * 128, (k + 1) * 128)
            p = jnp.exp2(s_ref[skip * 128:, hc] - m[:, hc]).astype(BF)
            off = 2 * k
            lpos = (off + DH) % DV
            r0 = pl.multiple_of(72 * g + (DH * k) // 8 * 8, 8)
            vw = vta[pl.ds(r0, DV), t0 + 128 - nk:t0 + 128]
            vw = jnp.where(rowv == lpos, 1.0, vw)
            acc = _nn(vw, p)
            val = acc * (1.0 / acc[lpos:lpos + 1, :])
            keep = (rows >= off) & (rows < off + DH)
            old = ota[pl.ds(r0, DV), t0:t0 + 128]
            ota[pl.ds(r0, DV), t0:t0 + 128] = jnp.where(keep, val, old)

    def a_group(g, ms, last=False):
        bufs = (sa0, sa1, sa2, sa3)
        ms = list(ms)
        for t in range(NT):
            if t + 2 < NT:
                ms.append(a_qk(g, t + 2, bufs[(t + 2) % 4]))
            elif not last:
                ms.append(a_qk(g + 1, t + 2 - NT, bufs[(t + 2) % 4]))
            a_pv(g, t, bufs[t % 4], ms[t])
        return tuple(ms[NT:])

    m_a = (a_qk(0, 0, sa0), a_qk(0, 1, sa1))
    m_a = lax.fori_loop(0, NG - 1, a_group, m_a)
    a_group(NG - 1, m_a, last=True)

    row24 = lax.broadcasted_iota(jnp.int32, (DV, QB), 0)

    def b_weights(item, ph):
        g = (item % H) // HG
        q0 = pl.multiple_of((item // H) * QB, QB)
        return _head_rows(qtb[g, :, pl.ds(q0, QB)], ph)

    def b_qk_chunk(c, wq, s_ref, m):
        st = _nn(kb[c * BK:(c + 1) * BK, :], wq)
        s_ref[c * BK:(c + 1) * BK, :] = st
        return jnp.maximum(m, jnp.max(st.reshape(BK // 8, 8, QB), axis=0))

    def b_finalize(item, ph, acc):
        q0 = pl.multiple_of((item // H) * QB, QB)
        h = item % H
        off = 2 * ph
        r0 = pl.multiple_of(((DH * h) // 8) * 8, 8)
        lpos = (off + DH) % DV
        l = acc[lpos:lpos + 1, :]
        val = acc * (1.0 / l)
        d = row24 - off
        keep = (d >= 0) & (d < DH)
        old = otb[pl.ds(r0, DV), pl.ds(q0, QB)]
        otb[pl.ds(r0, DV), pl.ds(q0, QB)] = jnp.where(keep, val, old)

    def b_step(item, ph, m_cur, s_cur, s_nxt=None):
        m_next = jnp.full((8, QB), NEG, F32)
        acc = jnp.zeros((DV, QB), F32)
        if s_nxt is not None:
            wq = b_weights(item + 1, (ph + 1) % HG)
        for c in range(S // BK):
            if s_nxt is not None:
                m_next = b_qk_chunk(c, wq, s_nxt, m_next)
            p = jnp.exp2(s_cur[c * BK:(c + 1) * BK, :] - m_cur)
            acc = acc + _nn(vtb[ph, :, c * BK:(c + 1) * BK], p.astype(BF))
        b_finalize(item, ph, acc)
        return jnp.max(m_next, axis=0, keepdims=True)

    wq0 = b_weights(0, 0)
    m_b = jnp.full((8, QB), NEG, F32)
    for cc in range(S // BK):
        m_b = b_qk_chunk(cc, wq0, sb0, m_b)
    m_b = jnp.max(m_b, axis=0, keepdims=True)

    def b_body(u, m):
        for k in range(0, B_UNROLL, 2):
            m = b_step(B_UNROLL * u + k, k % 4, m, sb0, sb1)
            m = b_step(B_UNROLL * u + k + 1, (k + 1) % 4, m, sb1, sb0)
        return m

    n_items = NQB * H
    n_loop = (n_items - 2) // B_UNROLL
    m_b = lax.fori_loop(0, n_loop, b_body, m_b)
    for k in range(n_loop * B_UNROLL, n_items - 2, 2):
        m_b = b_step(k, k % 4, m_b, sb0, sb1)
        m_b = b_step(k + 1, (k + 1) % 4, m_b, sb1, sb0)
    m_b = b_step(n_items - 2, (n_items - 2) % 4, m_b, sb0, sb1)
    b_step(n_items - 1, (n_items - 1) % 4, m_b, sb1)

    def out_piece(n, q0, nq):
        res = []
        for wo, ot in ((wota, ota), (wotb, otb)):
            o = ot[:, pl.ds(q0, nq)].astype(BF)
            res.append(_nn(wo[...], o).astype(BF))
        outv[pl.ds(q0, nq), :] = jnp.concatenate(res, axis=0).T
        out_dma(n, q0, nq).start()

    def out_dma(n, q0, nq):
        return pltpu.make_async_copy(outv.at[pl.ds(q0, nq), :], out_hbm.at[pl.ds(q0, nq), :], osems.at[n])

    def out_body(n, carry):
        out_piece(n, pl.multiple_of(n * QB, QB), QB)
        return carry

    lax.fori_loop(0, NQB - 1, out_body, 0)
    for n, (q0, nq) in enumerate(OUT_TAIL):
        pl.when(z_ref[0] == 0)(functools.partial(out_piece, NQB - 1 + n, q0, nq))
    for n in range(NQB - 1):
        out_dma(n, n * QB, QB).wait()
    for n, (q0, nq) in enumerate(OUT_TAIL):
        out_dma(NQB - 1 + n, q0, nq).wait()


@jax.jit
def pallas_concat_heads__sliding_block__grouped_kv_mqa__prompt_kernel(
    A_x: jax.Array,
    A_wqkv: jax.Array,
    A_wo: jax.Array,
    B_x: jax.Array,
    B_wq: jax.Array,
    B_wk: jax.Array,
    B_wv: jax.Array,
    B_wo: jax.Array,
):
    xa = A_x.reshape(S, D).T
    xb = B_x.reshape(S, D).T
    zeros = np.zeros((4,), np.int32)
    hbm = pl.BlockSpec(memory_space=pltpu.HBM)
    scratch = [
        pltpu.VMEM((D, S), BF),
        pltpu.VMEM((D, S), BF),
        pltpu.VMEM((D, 3 * D), BF),
        pltpu.VMEM((D, D), BF),
        pltpu.VMEM((D, D), BF),
        pltpu.VMEM((DH, D), BF),
        pltpu.VMEM((DH, D), BF),
        pltpu.VMEM((D, D), BF),
        pltpu.SemaphoreType.DMA((14,)),
        pltpu.SemaphoreType.DMA((NQB - 1 + len(OUT_TAIL),)),
        pltpu.VMEM((3 * D, D), BF),
        pltpu.VMEM((D, D), BF),
        pltpu.VMEM((D, D), BF),
        pltpu.VMEM((NG, S, GR), BF),
        pltpu.VMEM((D, S), F32),
        pltpu.VMEM((NG, GR, S), BF),
        pltpu.VMEM((NG, GR, S), BF),
        pltpu.VMEM((S, GR), BF),
        pltpu.VMEM((4, DV, S), F32),
        pltpu.VMEM((D, S), F32),
        pltpu.VMEM((D, S), F32),
        pltpu.VMEM((3 * 128, 128), F32),
        pltpu.VMEM((3 * 128, HG * 128), F32),
        pltpu.VMEM((3 * 128, HG * 128), F32),
        pltpu.VMEM((3 * 128, HG * 128), F32),
        pltpu.VMEM((3 * 128, HG * 128), F32),
        pltpu.VMEM((S, QB), F32),
        pltpu.VMEM((S, QB), F32),
        pltpu.VMEM((S, 2 * D), BF),
    ]
    out = pl.pallas_call(
        _kernel,
        in_specs=[pl.BlockSpec(memory_space=pltpu.SMEM)] + [hbm] * 8,
        out_specs=hbm,
        out_shape=jax.ShapeDtypeStruct((S, 2 * D), BF),
        scratch_shapes=scratch,
        compiler_params=pltpu.CompilerParams(vmem_limit_bytes=100 * 1024 * 1024),
    )(zeros, xa, xb, A_wqkv, A_wo, B_wq, B_wk.T, B_wv.T, B_wo)
    return out.reshape(1, S, 2 * D)
```
